```python
import jax
import jax.numpy as jnp

def _softmax(x, axis=-1):
    return jax.nn.softmax(x, axis=axis)

def _gelu(x):
    return jax.nn.gelu(x, approximate=True)

def _silu(x):
    return jax.nn.silu(x)

def _sigmoid(x):
    return jax.nn.sigmoid(x)

def _layernorm(x, axis=-1, eps=1e-05):
    m = jnp.mean(x, axis=axis, keepdims=True)
    v = jnp.var(x, axis=axis, keepdims=True)
    return (x - m) / jnp.sqrt(v + eps)

def _scatter_add(tgt, idx, src, axis=0):
    return tgt.at[idx].add(src)

def _segment_sum(src, seg, n):
    return jax.ops.segment_sum(src, seg, n)

class _Rng:

    def __init__(self, key):
        self._k = key

    def _next(self):
        self._k, sub = jax.random.split(self._k)
        return sub

    def normal(self, shape):
        return jax.random.normal(self._next(), shape, dtype=jnp.bfloat16)

    def randint(self, lo, hi, shape):
        return jax.random.randint(self._next(), shape, lo, hi, dtype=jnp.int32)

    def uniform(self, shape, lo=0.0, hi=1.0):
        return jax.random.uniform(self._next(), shape, jnp.bfloat16, lo, hi)

    def permutation(self, n):
        return jax.random.permutation(self._next(), n)
kernel_name = 'sequential_preLN__memory_aug_infini_attn__moe_arch_mod__prompt'

def setup_inputs():
    _rng = _Rng(jax.random.key(int.from_bytes(__import__("os").urandom(4), "little")))
    _w = lambda a: (lambda t: t.astype(jnp.bfloat16) if jnp.issubdtype(t.dtype, jnp.floating) else t)(jnp.asarray(a))

    def _A_setup():
        B, S, D, H = (1, 2048, 576, 32)
        N = 4
        L = max(1, S // N)
        sc = D ** (-0.5)
        return {'x': _w((lambda *s: _rng.normal(s) * 0.05)(B, N * L, D)), 'wq': _w((lambda *s: _rng.normal(s) * 0.05)(D, D) * sc), 'wk': _w((lambda *s: _rng.normal(s) * 0.05)(D, D) * sc), 'wv': _w((lambda *s: _rng.normal(s) * 0.05)(D, D) * sc), 'wo': _w((lambda *s: _rng.normal(s) * 0.05)(D, D) * sc), 'beta': _w((lambda *s: _rng.normal(s) * 0.05)(H))}
    _A_in = _A_setup()

    def _B_setup():
        B, S, D, F, C = (1, 2048, 576, 4608, 1)
        return {'x': _w((lambda *s: _rng.normal(s) * 0.05)(B, S, D)), 'w_r': _w((lambda *s: _rng.normal(s) * 0.05)(D)), 'w_gate': _w((lambda *s: _rng.normal(s) * 0.05)(D, F)), 'w_up': _w((lambda *s: _rng.normal(s) * 0.05)(D, F)), 'w_down': _w((lambda *s: _rng.normal(s) * 0.05)(F, D))}
    _B_in = _B_setup()
    return {'A_x': _A_in['x'], 'A_wq': _A_in['wq'], 'A_wk': _A_in['wk'], 'A_wv': _A_in['wv'], 'A_wo': _A_in['wo'], 'A_beta': _A_in['beta'], 'B_x': _B_in['x'], 'B_w_r': _B_in['w_r'], 'B_w_gate': _B_in['w_gate'], 'B_w_up': _B_in['w_up'], 'B_w_down': _B_in['w_down']}

def reference(A_x, A_wq, A_wk, A_wv, A_wo, A_beta, B_x, B_w_r, B_w_gate, B_w_up, B_w_down):

    def _A_ref(x, wq, wk, wv, wo, beta):
        B, S, D = x.shape
        H = 32
        Dh = D // H
        N = 4
        L = S // N
        q = (lambda x, *d: x.transpose(*d))((x @ wq).reshape(B, S, H, Dh), 0, 2, 1, 3).reshape(B, H, N, L, Dh)
        k = (lambda x, *d: x.transpose(*d))((x @ wk).reshape(B, S, H, Dh), 0, 2, 1, 3).reshape(B, H, N, L, Dh)
        v = (lambda x, *d: x.transpose(*d))((x @ wv).reshape(B, S, H, Dh), 0, 2, 1, 3).reshape(B, H, N, L, Dh)
        phi = lambda t: jnp.where(t > 0, t + 1.0, jnp.exp(t))
        scale = Dh ** (-0.5)
        ar = jnp.arange(L)
        mask = (lambda x, dt: x.astype(dt))(ar[:, None] < ar[None, :], x.dtype) * -1000000000.0
        g = _sigmoid(beta).reshape(1, H, 1, 1)
        M = jnp.einsum('bhd,bhe->bhde', q[:, :, 0, 0, :] * 0.0, q[:, :, 0, 0, :] * 0.0)
        z = q[:, :, 0, 0, :] * 0.0
        outs = []
        for s in range(N):
            qs, ks, vs = (q[:, :, s].copy(), k[:, :, s].copy(), v[:, :, s].copy())
            logits = jnp.einsum('bhqd,bhkd->bhqk', qs, ks) * scale + mask
            p = _softmax(logits, axis=-1)
            a_dot = jnp.einsum('bhqk,bhkd->bhqd', p, vs)
            pq = phi(qs)
            num = jnp.einsum('bhld,bhde->bhle', pq, M)
            den = jnp.einsum('bhld,bhd->bhl', pq, z)[..., None] + 1e-06
            a_mem = num / den
            o = g * a_mem + (1.0 - g) * a_dot
            outs.append(o)
            pk = phi(ks)
            M = M + jnp.einsum('bhld,bhle->bhde', pk, vs)
            z = z + jnp.einsum('bhld->bhd', pk)
        o = (lambda x, *d: x.transpose(*d))(jnp.stack(outs, 2).reshape(B, H, S, Dh), 0, 2, 1, 3).reshape(B, S, D)
        return o @ wo

    def _B_ref(x, w_r, w_gate, w_up, w_down):
        B, S, D = x.shape
        C = 1
        r = x @ w_r
        idx = jnp.argsort(-r, axis=-1)[:, :C]
        idx_e = jnp.repeat(idx.reshape(B, C, 1), D, axis=2)
        x_sel = jnp.take_along_axis(x, idx_e, axis=1)
        g = _silu(x_sel @ w_gate)
        u = x_sel @ w_up
        y = g * u @ w_down
        r_sel = _sigmoid(jnp.take_along_axis(r, idx, axis=1))
        y = y * r_sel.reshape(B, C, 1)
        b_off = (jnp.arange(B) * S).reshape(B, 1)
        flat_idx = (idx + b_off).reshape(B * C)
        zero = (x * 0.0).reshape(B * S, D)
        upd = _scatter_add(zero, flat_idx, y.reshape(B * C, D), axis=0)
        return x + upd.reshape(B, S, D)
    x = A_x
    h = x + _A_ref(_layernorm(x, axis=-1), A_wq, A_wk, A_wv, A_wo, A_beta)
    h2 = h + _B_ref(_layernorm(h, axis=-1), B_w_r, B_w_gate, B_w_up, B_w_down)
    return h2
```

```python
import jax
import jax.numpy as jnp
import numpy as np
from jax import lax
import jax.experimental.pallas as pl
import jax.experimental.pallas.tpu as pltpu

S, D, H, DH, NSEG, L = 2048, 576, 32, 18, 4, 512
F = 4608
NG = 5
HPG = 7
BF = jnp.bfloat16
F32 = jnp.float32
I32 = jnp.int32
NEG = -1e9 * 1.4426950408889634
QSCALE = float(DH ** -0.5 * 1.4426950408889634)
ONES = 0x3F803F80


def _dg(a, b):
    return lax.dot_general(a, b, (((1,), (1,)), ((), ())), preferred_element_type=F32)


def _mm(a, b):
    return jnp.dot(a, b, preferred_element_type=F32)


def _iota(shape, d):
    return lax.broadcasted_iota(I32, shape, d)


def _ln0(xf):
    m = jnp.sum(xf, axis=0, keepdims=True) * (1.0 / D)
    xc = xf - m
    v = jnp.sum(xc * xc, axis=0, keepdims=True) * (1.0 / D)
    return xc * lax.rsqrt(v + 1e-5)


def _phi(t):
    return jnp.where(t > 0, t + 1.0, jnp.exp(t))


def _r0(h):
    return (DH * h) // 16 * 16


GBASE = [(126 * g) // 16 * 16 for g in range(NG)]
GROWS = [144, 144, 144, 144, 80]


def _kernel(xt_hbm, wq_hbm, wk_hbm, wv_hbm, wo_hbm, beta_hbm, wr_hbm, wg_hbm, wu_hbm, wdt_hbm,
            out_hbm,
            xbuf, wraw, wqt, wkt, wvt, wot, beta_s, wr_s, wrc, q_s, k_s, pq_s, pk_s, vt_s, s_scr, m_scr,
            macc, zacc, mz, ot, hbuf, obuf, gv, wg, wu, wdt, best_v, best_i, fix,
            sem_x, sem_o, sem_w, sem_p, sem_f):
    def x_copy(s):
        return pltpu.make_async_copy(xt_hbm.at[:, pl.ds(s * L, L)], xbuf.at[:, pl.ds(s * L, L)], sem_x.at[s])

    def o_copy(s):
        return pltpu.make_async_copy(obuf.at[:, pl.ds(s * L, L)], out_hbm.at[:, pl.ds(s * L, L)], sem_o.at[s])

    w_copies = [pltpu.make_async_copy(wg_hbm, wg, sem_w.at[0]),
                pltpu.make_async_copy(wu_hbm, wu, sem_w.at[1]),
                pltpu.make_async_copy(wdt_hbm, wdt, sem_w.at[2])]
    p_copies = [pltpu.make_async_copy(src, wraw.at[n], sem_p.at[n])
                for n, src in enumerate((wq_hbm, wk_hbm, wv_hbm, wo_hbm))]
    p_copies.append(pltpu.make_async_copy(beta_hbm, beta_s, sem_p.at[4]))
    p_copies.append(pltpu.make_async_copy(wr_hbm, wr_s, sem_p.at[5]))
    for c in p_copies[:3]:
        c.start()
    x_copy(0).start()
    for c in p_copies[3:]:
        c.start()
    for s in range(1, NSEG):
        x_copy(s).start()
    for c in w_copies:
        c.start()

    for n, dst in ((0, wqt), (1, wkt)):
        p_copies[n].wait()
        wt32 = pltpu.bitcast(wraw[n].T, I32)
        for g in range(NG):
            nw = 63 if g < NG - 1 else (H - HPG * (NG - 1)) * DH // 2
            blk = jnp.concatenate([wt32[63 * g:63 * g + nw], jnp.zeros((64 - nw, D), I32)], axis=0)
            dst[pl.ds(128 * g, 128), :] = pltpu.bitcast(blk, BF)
    p_copies[2].wait()
    wvt[...] = wraw[2].T
    p_copies[3].wait()
    wot[...] = wraw[3].T
    p_copies[4].wait()
    p_copies[5].wait()

    gb = jax.nn.sigmoid(beta_s[...].reshape(1, H).astype(F32))
    for h in range(H):
        gv[h] = jnp.broadcast_to(gb[:, h:h + 1], (8, 128))
    wrc[...] = jnp.broadcast_to(wr_s[...].reshape(1, D), (128, D)).T.astype(F32)

    macc[...] = jnp.zeros(macc.shape, F32)
    zacc[...] = jnp.zeros(zacc.shape, F32)
    best_v[...] = jnp.full(best_v.shape, -jnp.inf, F32)
    best_i[...] = jnp.zeros(best_i.shape, I32)

    lane128 = _iota((128, 128), 1)
    kidx128 = _iota((128, 128), 0)
    causal = kidx128 <= lane128
    row16 = _iota((16, 128), 0)
    row8 = _iota((8, 128), 0)
    lane8 = _iota((8, 128), 1)

    def head_info(h):
        g = h // HPG
        off = DH * (h - HPG * g)
        r0 = _r0(h)
        o = DH * h - r0
        return g, off, r0, o

    def phase_proj(s):
        base = pl.multiple_of(s * L, L)
        for c in range(4):
            cols = pl.ds(base + 128 * c, 128)
            xnt = _ln0(xbuf[:, cols].astype(F32)).astype(BF)
            cc = pl.ds(128 * c, 128)
            for g in range(NG):
                gr = pl.ds(128 * g, 128)
                qf = _mm(wqt[gr, :], xnt)
                q_s[gr, cc] = (qf * QSCALE).astype(BF)
                pq_s[gr, cc] = _phi(qf).astype(BF)
                kb = _mm(wkt[gr, :], xnt).astype(BF).T
                k_s[g, cc, :] = kb
                pk_s[g, cc, :] = _phi(kb.astype(F32)).astype(BF)
            for t in range(4):
                vr = pl.ds(144 * t, 144)
                vt_s[vr, cc] = _mm(wvt[vr, :], xnt).astype(BF)

    def build_mz():
        for h in range(H):
            g, off, r0, o = head_info(h)
            u = h - HPG * g
            lm = (lane8 >= off) & (lane8 < off + DH)
            zsum = jnp.sum(zacc[g], axis=0, keepdims=True)
            zrow = jnp.where(lm, jnp.broadcast_to(zsum, (8, 128)), 0.0)
            parts = []
            for t in range(4):
                lo = 8 * t
                mt = macc[g, pl.ds(r0 - GBASE[g] + lo, 8), :]
                inh = (row8 + lo >= o) & (row8 + lo < o + DH)
                parts.append(jnp.where(inh, jnp.where(lm, mt, 0.0), zrow))
            mz[g, pl.ds(32 * u, 32), :] = jnp.concatenate(parts, axis=0).astype(BF)

    def update_mem():
        for g in range(NG):
            n = GROWS[g]
            acc = None
            zs = None
            for j in range(4):
                pk = pk_s[g, pl.ds(128 * j, 128), :]
                d = _mm(vt_s[pl.ds(GBASE[g], n), pl.ds(128 * j, 128)], pk)
                acc = d if acc is None else acc + d
                zj = jnp.sum(pk.astype(F32).reshape(16, 8, 128), axis=0)
                zs = zj if zs is None else zs + zj
            macc[g, pl.ds(0, n), :] += acc
            zacc[g] += zs

    def stage_a(h, u, i, slot):
        g, off, r0, o = head_info(h)
        w0, w1 = off // 2, off // 2 + DH // 2
        parts = []
        for t in range(8):
            if 8 * t + 8 <= w0 or 8 * t >= w1:
                parts.append(jnp.zeros((8, 128), I32))
            else:
                v = pltpu.bitcast(q_s[pl.ds(128 * g + 16 * t, 16), pl.ds(128 * i, 128)], I32)
                keep = (row8 + 8 * t >= w0) & (row8 + 8 * t < w1)
                parts.append(jnp.where(keep, v, 0))
        qi = pltpu.bitcast(jnp.concatenate(parts, axis=0), BF)
        mm = None
        for j in range(i + 1):
            s = _mm(k_s[g, pl.ds(128 * j, 128), :], qi)
            if j == i:
                s = jnp.where(causal, s, s + NEG)
            s_scr[slot, u, pl.ds(128 * j, 128), :] = s
            mm = s if mm is None else jnp.maximum(mm, s)
        m = jnp.max(mm, axis=0, keepdims=True)
        m_scr[slot, u] = jnp.broadcast_to(m, (8, 128))

    def stage_b(h, u, i, slot):
        g, off, r0, o = head_info(h)
        ug = h - HPG * g
        m = m_scr[slot, u]
        m = jnp.concatenate([m] * 16, axis=0)
        rm = (row16 >= o // 2) & (row16 < o // 2 + DH // 2)
        acc = None
        for j in range(i + 1):
            vt = pltpu.bitcast(vt_s[pl.ds(r0, 32), pl.ds(128 * j, 128)], I32)
            vt1 = pltpu.bitcast(jnp.where(rm, vt, ONES), BF)
            p = jnp.exp2(s_scr[slot, u, pl.ds(128 * j, 128), :] - m).astype(BF)
            pv = _mm(vt1, p)
            acc = pv if acc is None else acc + pv
        mem = _mm(mz[g, pl.ds(32 * ug, 32), :], pq_s[pl.ds(128 * g, 128), pl.ds(128 * i, 128)])
        lsel = 0 if o >= 8 else 24
        gh = gv[h]
        a = (1.0 - gh) / acc[lsel:lsel + 8]
        b = gh / (mem[lsel:lsel + 8] + 1e-6)
        res = {}
        for t in range(4):
            lo = 8 * t
            if lo + 8 <= o or lo >= o + DH:
                continue
            res[r0 + lo] = acc[lo:lo + 8] * a + mem[lo:lo + 8] * b
        return res

    def merge_quad(qd, i, results):
        for t in range(9):
            row = 72 * qd + 8 * t
            val = None
            for u in range(4):
                h = 4 * qd + u
                lo, hi = DH * h, DH * h + DH
                if row + 8 <= lo or row >= hi:
                    continue
                v = results[u][row]
                if val is None:
                    val = v
                else:
                    val = jnp.where(row8 + row >= lo, v, val)
            ot[pl.ds(row, 8), pl.ds(128 * i, 128)] = val

    def phase_attn():
        steps = [(qd, i) for qd in range(8) for i in range(4)]
        for t in range(len(steps) + 1):
            res = []
            for u in range(4):
                if t < len(steps):
                    qd, i = steps[t]
                    stage_a(4 * qd + u, u, i, t % 2)
                if t > 0:
                    qd, i = steps[t - 1]
                    res.append(stage_b(4 * qd + u, u, i, (t - 1) % 2))
            if t > 0:
                qd, i = steps[t - 1]
                merge_quad(qd, i, res)

    def phase_out(s):
        base = pl.multiple_of(s * L, L)
        for c in range(4):
            cols = pl.ds(base + 128 * c, 128)
            oc = ot[:, pl.ds(128 * c, 128)].astype(BF)
            attn = jnp.concatenate([_mm(wot[pl.ds(144 * t, 144), :], oc) for t in range(4)], axis=0)
            hb = (xbuf[:, cols].astype(F32) + attn.astype(BF).astype(F32)).astype(BF)
            hbuf[:, cols] = hb
            hf = hb.astype(F32)
            lnf = _ln0(hf).astype(BF).astype(F32)
            obuf[:, cols] = (hf + lnf).astype(BF)
            r = jnp.sum(lnf * wrc[...], axis=0, keepdims=True).astype(BF).astype(F32)
            rt = jnp.broadcast_to(r, (8, 128))
            bv = best_v[...]
            better = rt > bv
            best_v[...] = jnp.where(better, rt, bv)
            best_i[...] = jnp.where(better, lane8 + (base + 128 * c), best_i[...])

    def seg_body(s, carry):
        x_copy(s).wait()
        phase_proj(s)
        build_mz()
        phase_attn()
        update_mem()
        phase_out(s)
        o_copy(s).start()
        return carry

    lax.fori_loop(0, NSEG, seg_body, 0)

    bv = best_v[...]
    bmax = jnp.max(bv, axis=1, keepdims=True)
    cand = jnp.where(bv == bmax, best_i[...], S)
    sel = jnp.clip(jnp.min(cand), 0, S - 1)
    cstart = pl.multiple_of(sel // 128 * 128, 128)
    cols = pl.ds(cstart, 128)
    hf = hbuf[:, cols].astype(F32)
    lnb = _ln0(hf).astype(BF)
    onehot = jnp.where(_iota((16, 128), 1) == sel - cstart, 1.0, 0.0).astype(BF)
    xs = _dg(onehot, lnb).astype(BF)
    for c in w_copies:
        c.wait()
    gate = _mm(xs, wg[...])[0:8].astype(BF).astype(F32)
    up = _mm(xs, wu[...])[0:8].astype(BF).astype(F32)
    act = (gate * jax.nn.sigmoid(gate)).astype(BF).astype(F32)
    hid = (act * up).astype(BF)
    hid = jnp.concatenate([hid, hid], axis=0)
    y = _dg(hid, wdt[...])[0:8].astype(BF).astype(F32)
    y = (y * jax.nn.sigmoid(bmax).astype(BF).astype(F32)).astype(BF)
    yt = jnp.broadcast_to(y[0:1], (128, D)).T.astype(F32)
    new = (hf + (lnb.astype(F32) + yt).astype(BF).astype(F32)).astype(BF)
    for s in range(NSEG):
        o_copy(s).wait()
    fix[...] = jnp.where(_iota((D, 128), 1) == sel - cstart, new, obuf[:, cols])
    cp = pltpu.make_async_copy(fix, out_hbm.at[:, cols], sem_f)
    cp.start()
    cp.wait()


@jax.jit
def pallas_sequential_preLN__memory_aug_infini_attn__moe_arch_mod__prompt_kernel(
    A_x, A_wq, A_wk, A_wv, A_wo, A_beta, B_x, B_w_r, B_w_gate, B_w_up, B_w_down,
):
    del B_x
    hbm = pl.BlockSpec(memory_space=pltpu.HBM)
    V = pltpu.VMEM
    out_t = pl.pallas_call(
        _kernel,
        in_specs=[hbm] * 10,
        out_specs=hbm,
        out_shape=jax.ShapeDtypeStruct((D, S), BF),
        scratch_shapes=[
            V((D, S), BF),
            V((4, D, D), BF),
            V((640, D), BF), V((640, D), BF), V((D, D), BF), V((D, D), BF),
            V((H,), BF), V((D,), BF), V((D, 128), F32),
            V((640, L), BF), V((NG, L, 128), BF), V((640, L), BF), V((NG, L, 128), BF),
            V((D, L), BF),
            V((2, 4, L, 128), F32), V((2, 4, 8, 128), F32),
            V((NG, 144, 128), F32), V((NG, 8, 128), F32), V((NG, 224, 128), BF),
            V((D, L), F32),
            V((D, S), BF), V((D, S), BF),
            V((H, 8, 128), F32),
            V((D, F), BF), V((D, F), BF), V((D, F), BF),
            V((8, 128), F32), V((8, 128), I32),
            V((D, 128), BF),
            pltpu.SemaphoreType.DMA((NSEG,)), pltpu.SemaphoreType.DMA((NSEG,)),
            pltpu.SemaphoreType.DMA((3,)), pltpu.SemaphoreType.DMA((6,)), pltpu.SemaphoreType.DMA(()),
        ],
        compiler_params=pltpu.CompilerParams(vmem_limit_bytes=100 * 2**20),
    )(A_x.reshape(S, D).T, A_wq, A_wk, A_wv, A_wo, A_beta, B_w_r, B_w_gate, B_w_up, B_w_down.T)
    return out_t.T.reshape(1, S, D)
```

```python
import jax
import jax.numpy as jnp
import numpy as np
from jax import lax
import jax.experimental.pallas as pl
import jax.experimental.pallas.tpu as pltpu

S, D, H, DH, NSEG, L = 2048, 576, 32, 18, 4, 512
F = 4608
NG = 5
HPG = 7
BF = jnp.bfloat16
F32 = jnp.float32
I32 = jnp.int32
NEG = -1e9 * 1.4426950408889634
QSCALE = float(DH ** -0.5 * 1.4426950408889634)
ONES = 0x3F803F80


def _dg(a, b):
    return lax.dot_general(a, b, (((1,), (1,)), ((), ())), preferred_element_type=F32)


def _mm(a, b):
    return jnp.dot(a, b, preferred_element_type=F32)


def _iota(shape, d):
    return lax.broadcasted_iota(I32, shape, d)


def _ln0(xf):
    m = jnp.sum(xf, axis=0, keepdims=True) * (1.0 / D)
    xc = xf - m
    v = jnp.sum(xc * xc, axis=0, keepdims=True) * (1.0 / D)
    return xc * lax.rsqrt(v + 1e-5)


def _phi(t):
    return jnp.where(t > 0, t + 1.0, jnp.exp(t))


def _rcp(x):
    r = pl.reciprocal(x, approx=True)
    return r * (2.0 - x * r)


def _r0(h):
    return (DH * h) // 16 * 16


GBASE = [(126 * g) // 16 * 16 for g in range(NG)]
GROWS = [144, 144, 144, 144, 80]


def _kernel(xt_hbm, wq_hbm, wk_hbm, wv_hbm, wo_hbm, beta_hbm, wr_hbm, wg_hbm, wu_hbm, wdt_hbm,
            out_hbm,
            xbuf, wraw, wqt, wkp, wvt, wot, beta_s, wr_s, wrc, q_s, k_s, memo, vt_s, s_scr, m_scr,
            cbias, macc, zacc, mz, ot, hbuf, obuf, gv, wg, wu, wdt, best_v, best_i, fix,
            sem_x, sem_o, sem_w, sem_p, sem_f):
    def x_copy(s):
        return pltpu.make_async_copy(xt_hbm.at[:, pl.ds(s * L, L)], xbuf.at[:, pl.ds(s * L, L)], sem_x.at[s])

    def o_copy(s):
        return pltpu.make_async_copy(obuf.at[:, pl.ds(s * L, L)], out_hbm.at[:, pl.ds(s * L, L)], sem_o.at[s])

    w_copies = [pltpu.make_async_copy(wg_hbm, wg, sem_w.at[0]),
                pltpu.make_async_copy(wu_hbm, wu, sem_w.at[1]),
                pltpu.make_async_copy(wdt_hbm, wdt, sem_w.at[2])]
    p_copies = [pltpu.make_async_copy(src, wraw.at[n], sem_p.at[n])
                for n, src in enumerate((wq_hbm, wk_hbm, wv_hbm, wo_hbm))]
    p_copies.append(pltpu.make_async_copy(beta_hbm, beta_s, sem_p.at[4]))
    p_copies.append(pltpu.make_async_copy(wr_hbm, wr_s, sem_p.at[5]))
    for c in p_copies[:3]:
        c.start()
    x_copy(0).start()
    for c in p_copies[3:]:
        c.start()

    for n, dst in ((0, wqt),):
        p_copies[n].wait()
        wt32 = pltpu.bitcast(wraw[n].T, I32)
        for g in range(NG):
            nw = 63 if g < NG - 1 else (H - HPG * (NG - 1)) * DH // 2
            blk = jnp.concatenate([wt32[63 * g:63 * g + nw], jnp.zeros((64 - nw, D), I32)], axis=0)
            dst[pl.ds(128 * g, 128), :] = pltpu.bitcast(blk, BF)
    p_copies[1].wait()
    lane96 = _iota((96, 128), 1)
    for r in range(0, D, 192):
        w32 = pltpu.bitcast(wraw[1, pl.ds(r, 192), :], I32)
        w32 = jnp.concatenate([w32, jnp.zeros((96, 64), I32)], axis=1)
        for g in range(NG):
            sh = 2 * g
            cur = w32[:, 128 * g:128 * g + 128]
            if g == 0:
                t = cur
            else:
                prv = w32[:, 128 * (g - 1):128 * g]
                t = jnp.where(lane96 < sh, pltpu.roll(prv, sh, 1), pltpu.roll(cur, sh, 1))
            nv = 126 if g < NG - 1 else (H - HPG * (NG - 1)) * DH
            t = jnp.where(lane96 < nv, t, 0)
            wkp[pl.ds(r, 192), pl.ds(128 * g, 128)] = pltpu.bitcast(t, BF)
    p_copies[2].wait()
    wvt[...] = wraw[2].T
    p_copies[3].wait()
    wot[...] = wraw[3].T
    p_copies[4].wait()
    p_copies[5].wait()
    for s in range(1, NSEG):
        x_copy(s).start()
    for c in w_copies:
        c.start()

    gb = jax.nn.sigmoid(beta_s[...].reshape(1, H).astype(F32))
    for h in range(H):
        gv[h] = jnp.broadcast_to(gb[:, h:h + 1], (8, 128))
    wrc[...] = jnp.broadcast_to(wr_s[...].reshape(1, D), (128, D)).T.astype(F32)

    macc[...] = jnp.zeros(macc.shape, F32)
    zacc[...] = jnp.zeros(zacc.shape, F32)
    best_v[...] = jnp.full(best_v.shape, -jnp.inf, F32)
    best_i[...] = jnp.zeros(best_i.shape, I32)

    lane128 = _iota((128, 128), 1)
    kidx128 = _iota((128, 128), 0)
    causal = kidx128 <= lane128
    cbias[...] = jnp.where(causal, 0.0, NEG)
    row16 = _iota((16, 128), 0)
    row8 = _iota((8, 128), 0)
    lane8 = _iota((8, 128), 1)

    def head_info(h):
        g = h // HPG
        off = DH * (h - HPG * g)
        r0 = _r0(h)
        o = DH * h - r0
        return g, off, r0, o

    def phase_proj(s):
        base = pl.multiple_of(s * L, L)
        for c in range(4):
            cols = pl.ds(base + 128 * c, 128)
            xnt = _ln0(xbuf[:, cols].astype(F32)).astype(BF)
            xnf = xnt.T
            cc = pl.ds(128 * c, 128)
            for g in range(NG):
                gr = pl.ds(128 * g, 128)
                qf = _mm(wqt[gr, :], xnt)
                q_s[gr, cc] = (qf * QSCALE).astype(BF)
                k_s[g, cc, :] = _mm(xnf, wkp[:, gr]).astype(BF)
            for t in range(4):
                vr = pl.ds(144 * t, 144)
                vt_s[vr, cc] = _mm(wvt[vr, :], xnt).astype(BF)

    def build_mz():
        for h in range(H):
            g, off, r0, o = head_info(h)
            u = h - HPG * g
            lm = (lane8 >= off) & (lane8 < off + DH)
            zsum = jnp.sum(zacc[g], axis=0, keepdims=True)
            zrow = jnp.where(lm, jnp.broadcast_to(zsum, (8, 128)), 0.0)
            parts = []
            for t in range(4):
                lo = 8 * t
                mt = macc[g, pl.ds(r0 - GBASE[g] + lo, 8), :]
                inh = (row8 + lo >= o) & (row8 + lo < o + DH)
                parts.append(jnp.where(inh, jnp.where(lm, mt, 0.0), zrow))
            mz[g, pl.ds(32 * u, 32), :] = jnp.concatenate(parts, axis=0).astype(BF)

    def phase_mem():
        for g in range(NG):
            n = 32 * (HPG if g < NG - 1 else H - HPG * (NG - 1))
            for i in range(4):
                qf = q_s[pl.ds(128 * g, 128), pl.ds(128 * i, 128)].astype(F32) * (1.0 / QSCALE)
                memo[g, i, pl.ds(0, n), :] = _mm(mz[g, pl.ds(0, n), :], _phi(qf).astype(BF))

    def update_mem():
        for g in range(NG):
            n = GROWS[g]
            acc = None
            zs = None
            for j in range(4):
                pk = _phi(k_s[g, pl.ds(128 * j, 128), :].astype(F32)).astype(BF)
                d = _mm(vt_s[pl.ds(GBASE[g], n), pl.ds(128 * j, 128)], pk)
                acc = d if acc is None else acc + d
                zj = jnp.sum(pk.astype(F32).reshape(16, 8, 128), axis=0)
                zs = zj if zs is None else zs + zj
            macc[g, pl.ds(0, n), :] += acc
            zacc[g] += zs

    def stage_a(h, u, i, slot):
        g, off, r0, o = head_info(h)
        w0, w1 = off // 2, off // 2 + DH // 2
        parts = []
        for t in range(8):
            if 8 * t + 8 <= w0 or 8 * t >= w1:
                parts.append(jnp.zeros((8, 128), I32))
            else:
                v = pltpu.bitcast(q_s[pl.ds(128 * g + 16 * t, 16), pl.ds(128 * i, 128)], I32)
                keep = (row8 + 8 * t >= w0) & (row8 + 8 * t < w1)
                parts.append(jnp.where(keep, v, 0))
        qi = pltpu.bitcast(jnp.concatenate(parts, axis=0), BF)
        mm = None
        for j in range(i + 1):
            s = _mm(k_s[g, pl.ds(128 * j, 128), :], qi)
            if j == i:
                s = s + cbias[...]
            s_scr[slot, u, pl.ds(128 * j, 128), :] = s
            mm = s if mm is None else jnp.maximum(mm, s)
        m = jnp.max(mm, axis=0, keepdims=True)
        m_scr[slot, u] = jnp.broadcast_to(m, (8, 128))

    def stage_b(h, u, i, slot):
        g, off, r0, o = head_info(h)
        ug = h - HPG * g
        m = m_scr[slot, u]
        m = jnp.concatenate([m] * 16, axis=0)
        rm = (row16 >= o // 2) & (row16 < o // 2 + DH // 2)
        acc = None
        for j in range(i + 1):
            vt = pltpu.bitcast(vt_s[pl.ds(r0, 32), pl.ds(128 * j, 128)], I32)
            vt1 = pltpu.bitcast(jnp.where(rm, vt, ONES), BF)
            p = jnp.exp2(s_scr[slot, u, pl.ds(128 * j, 128), :] - m).astype(BF)
            pv = _mm(vt1, p)
            acc = pv if acc is None else acc + pv
        mem = memo[g, i, pl.ds(32 * ug, 32), :]
        lsel = 0 if o >= 8 else 24
        gh = gv[h]
        lsum = acc[lsel:lsel + 8]
        den = mem[lsel:lsel + 8] + 1e-6
        a = (1.0 - gh) * _rcp(lsum)
        b = gh * _rcp(den)
        res = {}
        for t in range(4):
            lo = 8 * t
            if lo + 8 <= o or lo >= o + DH:
                continue
            res[r0 + lo] = acc[lo:lo + 8] * a + mem[lo:lo + 8] * b
        return res

    def merge_quad(qd, i, results):
        for t in range(9):
            row = 72 * qd + 8 * t
            val = None
            for u in range(4):
                h = 4 * qd + u
                lo, hi = DH * h, DH * h + DH
                if row + 8 <= lo or row >= hi:
                    continue
                v = results[u][row]
                if val is None:
                    val = v
                else:
                    val = jnp.where(row8 + row >= lo, v, val)
            ot[pl.ds(row, 8), pl.ds(128 * i, 128)] = val

    def phase_attn():
        steps = [(qd, i) for qd in range(8) for i in range(4)]
        for t in range(len(steps) + 1):
            res = []
            def A(u):
                if t < len(steps):
                    qd, i = steps[t]
                    stage_a(4 * qd + u, u, i, t % 2)
            def B(u):
                if t > 0:
                    qd, i = steps[t - 1]
                    res.append(stage_b(4 * qd + u, u, i, (t - 1) % 2))
            for u in range(4):
                A(u)
                B(u)
            if t > 0:
                qd, i = steps[t - 1]
                merge_quad(qd, i, res)

    def phase_out(s):
        base = pl.multiple_of(s * L, L)
        for c in range(4):
            cols = pl.ds(base + 128 * c, 128)
            oc = ot[:, pl.ds(128 * c, 128)].astype(BF)
            attn = jnp.concatenate([_mm(wot[pl.ds(144 * t, 144), :], oc) for t in range(4)], axis=0)
            hb = (xbuf[:, cols].astype(F32) + attn.astype(BF).astype(F32)).astype(BF)
            hbuf[:, cols] = hb
            hf = hb.astype(F32)
            lnf = _ln0(hf).astype(BF).astype(F32)
            obuf[:, cols] = (hf + lnf).astype(BF)
            r = jnp.sum(lnf * wrc[...], axis=0, keepdims=True).astype(BF).astype(F32)
            rt = jnp.broadcast_to(r, (8, 128))
            bv = best_v[...]
            better = rt > bv
            best_v[...] = jnp.where(better, rt, bv)
            best_i[...] = jnp.where(better, lane8 + (base + 128 * c), best_i[...])

    def seg_body(s, carry):
        x_copy(s).wait()
        phase_proj(s)
        build_mz()
        phase_mem()
        phase_attn()
        update_mem()
        phase_out(s)
        o_copy(s).start()
        return carry

    lax.fori_loop(0, NSEG, seg_body, 0)

    bv = best_v[...]
    bmax = jnp.max(bv, axis=1, keepdims=True)
    cand = jnp.where(bv == bmax, best_i[...], S)
    sel = jnp.clip(jnp.min(cand), 0, S - 1)
    cstart = pl.multiple_of(sel // 128 * 128, 128)
    cols = pl.ds(cstart, 128)
    hf = hbuf[:, cols].astype(F32)
    lnb = _ln0(hf).astype(BF)
    onehot = jnp.where(_iota((16, 128), 1) == sel - cstart, 1.0, 0.0).astype(BF)
    xs = _dg(onehot, lnb).astype(BF)
    for c in w_copies:
        c.wait()
    gate = _mm(xs, wg[...])[0:8].astype(BF).astype(F32)
    up = _mm(xs, wu[...])[0:8].astype(BF).astype(F32)
    act = (gate * jax.nn.sigmoid(gate)).astype(BF).astype(F32)
    hid = (act * up).astype(BF)
    hid = jnp.concatenate([hid, hid], axis=0)
    y = _dg(hid, wdt[...])[0:8].astype(BF).astype(F32)
    y = (y * jax.nn.sigmoid(bmax).astype(BF).astype(F32)).astype(BF)
    yt = jnp.broadcast_to(y[0:1], (128, D)).T.astype(F32)
    new = (hf + (lnb.astype(F32) + yt).astype(BF).astype(F32)).astype(BF)
    for s in range(NSEG):
        o_copy(s).wait()
    fix[...] = jnp.where(_iota((D, 128), 1) == sel - cstart, new, obuf[:, cols])
    cp = pltpu.make_async_copy(fix, out_hbm.at[:, cols], sem_f)
    cp.start()
    cp.wait()


@jax.jit
def pallas_sequential_preLN__memory_aug_infini_attn__moe_arch_mod__prompt_kernel(
    A_x, A_wq, A_wk, A_wv, A_wo, A_beta, B_x, B_w_r, B_w_gate, B_w_up, B_w_down,
):
    del B_x
    hbm = pl.BlockSpec(memory_space=pltpu.HBM)
    V = pltpu.VMEM
    out_t = pl.pallas_call(
        _kernel,
        in_specs=[hbm] * 10,
        out_specs=hbm,
        out_shape=jax.ShapeDtypeStruct((D, S), BF),
        scratch_shapes=[
            V((D, S), BF),
            V((4, D, D), BF),
            V((640, D), BF), V((D, 640), BF), V((D, D), BF), V((D, D), BF),
            V((H,), BF), V((D,), BF), V((D, 128), F32),
            V((640, L), BF), V((NG, L, 128), BF), V((NG, 4, 224, 128), F32),
            V((D, L), BF),
            V((2, 4, L, 128), F32), V((2, 4, 8, 128), F32),
            V((128, 128), F32),
            V((NG, 144, 128), F32), V((NG, 8, 128), F32), V((NG, 224, 128), BF),
            V((D, L), F32),
            V((D, S), BF), V((D, S), BF),
            V((H, 8, 128), F32),
            V((D, F), BF), V((D, F), BF), V((D, F), BF),
            V((8, 128), F32), V((8, 128), I32),
            V((D, 128), BF),
            pltpu.SemaphoreType.DMA((NSEG,)), pltpu.SemaphoreType.DMA((NSEG,)),
            pltpu.SemaphoreType.DMA((3,)), pltpu.SemaphoreType.DMA((6,)), pltpu.SemaphoreType.DMA(()),
        ],
        compiler_params=pltpu.CompilerParams(vmem_limit_bytes=100 * 2**20),
    )(A_x.reshape(S, D).T, A_wq, A_wk, A_wv, A_wo, A_beta, B_w_r, B_w_gate, B_w_up, B_w_down.T)
    return out_t.T.reshape(1, S, D)
```
